```python
import os as _os
_os.environ.setdefault("JAX_PLATFORMS", "cpu")
import jax
import jax.numpy as jnp

def _softmax(x, axis=-1):
    return jax.nn.softmax(x, axis=axis)
def _gelu(x):
    return jax.nn.gelu(x, approximate=True)
def _silu(x):
    return jax.nn.silu(x)
def _sigmoid(x):
    return jax.nn.sigmoid(x)
def _layernorm(x, axis=-1, eps=1e-5):
    m = jnp.mean(x, axis=axis, keepdims=True)
    v = jnp.var(x, axis=axis, keepdims=True)
    return (x - m) / jnp.sqrt(v + eps)
def _scatter_add(tgt, idx, src, axis=0):
    return tgt.at[idx].add(src)
def _segment_sum(src, seg, n):
    return jax.ops.segment_sum(src, seg, n)
class _Rng:
    def __init__(self, key):
        self._k = key
    def _next(self):
        self._k, sub = jax.random.split(self._k)
        return sub
    def normal(self, shape):
        return jax.random.normal(self._next(), shape, dtype=jnp.bfloat16)
    def randint(self, lo, hi, shape):
        return jax.random.randint(self._next(), shape, lo, hi, dtype=jnp.int32)
    def uniform(self, shape, lo=0.0, hi=1.0):
        return jax.random.uniform(self._next(), shape, jnp.bfloat16, lo, hi)
    def permutation(self, n):
        return jax.random.permutation(self._next(), n)


kernel_name = 'gated_mix__mha_block__softmax_full_mha__prompt'

def setup_inputs():
    _rng = _Rng(jax.random.key(int.from_bytes(__import__("os").urandom(4), "little")))
    _w = (lambda a: (lambda t: t.astype(jnp.bfloat16) if jnp.issubdtype(t.dtype, jnp.floating) else t)(jnp.asarray(a)))
    def _A_setup():
        B, S, D, H = 1, 2048, 448, 16
        return {
            "x": _w((lambda *s: _rng.normal(s) * 0.05)(B, S, D)),
            "wqkv": _w((lambda *s: _rng.normal(s) * 0.4)(D, 3 * D)),
            "wo": _w((lambda *s: _rng.normal(s) * 0.05)(D, D)),
        }
    _A_in = _A_setup()

    def _B_setup():
        B, S, D = 1, 2048, 448
        return {
            "x": _w((lambda *s: _rng.normal(s) * 0.05)(B, S, D)),
            "wqkv": _w((lambda *s: _rng.normal(s) * 0.4)(D, 3 * D)),
            "wo": _w((lambda *s: _rng.normal(s) * 0.05)(D, D)),
        }
    _B_in = _B_setup()

    return {
        "A_x": _A_in["x"],
        "A_wqkv": _A_in["wqkv"],
        "A_wo": _A_in["wo"],
        "B_x": _B_in["x"],
        "B_wqkv": _B_in["wqkv"],
        "B_wo": _B_in["wo"],
        "gate_w": _w((lambda *s: _rng.normal(s) * 0.05)(448) * 16.0),
    }

def reference(A_x, A_wqkv, A_wo, B_x, B_wqkv, B_wo, gate_w):
    def _A_ref(x, wqkv, wo):
        B, S, D = x.shape
        H = 16
        Dh = D // H
        qkv = (lambda x, *d: x.transpose(*d))((x @ wqkv).reshape(B, S, 3, H, Dh), 2, 0, 3, 1, 4)
        q, k, v = qkv[0], qkv[1], qkv[2]
        scores = jnp.einsum("bhqd,bhkd->bhqk", q, k) * (Dh ** -0.5)
        p = _softmax(scores, axis=-1)
        o = jnp.einsum("bhqk,bhkd->bhqd", p, v)
        return (lambda x, *d: x.transpose(*d))(o, 0, 2, 1, 3).reshape(B, S, D) @ wo

    def _B_ref(x, wqkv, wo):
        B, S, D = x.shape
        H = 16; Dh = D // H
        qkv = (lambda x, *d: x.transpose(*d))((x @ wqkv).reshape(B, S, 3, H, Dh), 2, 0, 3, 1, 4)
        q, k, v = qkv[0], qkv[1], qkv[2]
        scale = Dh ** -0.5
        scores = jnp.einsum("bhqd,bhkd->bhqk", q, k) * scale
        p = _softmax(scores, axis=-1)
        o = jnp.einsum("bhqk,bhkd->bhqd", p, v)
        return (lambda x, *d: x.transpose(*d))(o, 0, 2, 1, 3).reshape(B, S, D) @ wo

    x = A_x
    g = _sigmoid((x * gate_w).sum(-1, keepdims=True))
    a = _A_ref(x, A_wqkv, A_wo)
    b = _B_ref(x, B_wqkv, B_wo)
    return g * a + (1 - g) * b
```

```python
import functools

import jax
import jax.numpy as jnp
import numpy as np
from jax import lax
import jax.experimental.pallas as pl
import jax.experimental.pallas.tpu as pltpu

S = 2048
D = 448
H = 16
DH = 28
HP = 32
NH = 2 * H
SLAB = 4 * DH
AUG = SLAB
BQ = 1024
CK = 512
CKS = 256
TC = 512
QROWS = D + 16
LOG2E = float(np.log2(np.e))
QSCALE = float(DH ** -0.5) * LOG2E
L_MIN = float(2.0 ** -40)
L_MAX = float(2.0 ** 20)

bf16 = jnp.bfloat16
f32 = jnp.float32


def _mm(a, b):
    return jnp.dot(a, b, preferred_element_type=f32)


def _space_heads(w):
    z = jnp.zeros((HP - DH, w.shape[1]), w.dtype)
    parts = []
    for h in range(H):
        parts += [w[DH * h:DH * (h + 1)], z]
    return jnp.concatenate(parts, axis=0)


def _prologue(x_ref, w_refs, wo_refs, gw_ref, qt_scr, k_scr, vt_scr, wot_scr, m_scr, g_scr, wt_scr):
    qt_scr[:, D:QROWS, :] = jnp.zeros((2, QROWS - D, S), bf16)
    gl = jnp.broadcast_to(gw_ref[...].reshape(1, D), (16, D))
    for t in range(0, S, TC):
        gs = _mm(gl, x_ref[:, t:t + TC])[0:8]
        g = 1.0 / (1.0 + jnp.exp(-gs))
        g_scr[0, :, t:t + TC] = g
        g_scr[1, :, t:t + TC] = 1.0 - g

    row_v = lax.broadcasted_iota(jnp.int32, (H * HP, TC), 0) % HP
    row_k = lax.broadcasted_iota(jnp.int32, (128, TC), 0)
    for br in range(2):
        wt = w_refs[br][...].astype(f32).T
        wt_scr[0:2 * D, :] = wt[0:2 * D].astype(bf16)
        wt_scr[2 * D:2 * D + H * HP, :] = _space_heads(wt[2 * D:3 * D]).astype(bf16)
        wo = _space_heads(wo_refs[br][...].astype(f32))
        wot_scr[:, br * H * HP:(br + 1) * H * HP] = wo.T.astype(bf16)

        kmax = [None] * H
        for t in range(0, S, TC):
            xt = x_ref[:, t:t + TC]
            kt = _mm(wt_scr[D:2 * D + 16, :], xt)
            k2 = kt * kt
            for h in range(H):
                n2 = jnp.sum(k2[DH * h:DH * (h + 1)], axis=0, keepdims=True)
                kmax[h] = n2 if kmax[h] is None else jnp.maximum(kmax[h], n2)
            for s in range(4):
                slab = jnp.where(row_k == AUG, 1.0, kt[SLAB * s:SLAB * s + 128])
                k_scr[br * 4 + s, t:t + TC, :] = slab.T.astype(bf16)
            vt = _mm(wt_scr[2 * D:2 * D + H * HP, :], xt)
            vt = jnp.where(row_v == DH, 1.0, vt)
            vt_scr[br * H * HP:(br + 1) * H * HP, t:t + TC] = vt.astype(bf16)
        kmax = [jnp.max(k, axis=1, keepdims=True) for k in kmax]
        for t in range(0, S, TC):
            xt = x_ref[:, t:t + TC]
            qt = _mm(wt_scr[0:D, :], xt) * QSCALE
            qt_scr[br, 0:D, t:t + TC] = qt.astype(bf16)
            q2 = qt * qt
            ms = []
            for h in range(H):
                n2 = jnp.sum(q2[DH * h:DH * (h + 1)], axis=0, keepdims=True)
                ms.append(n2 * kmax[h])
            m = jnp.sqrt(jnp.concatenate(ms, axis=0)) * (1.0 + 2.0 ** -6)
            m_scr[br * H:(br + 1) * H, t:t + TC] = m


def _attend(fast, q0, qt_scr, k_scr, vt_scr, m_scr, g_scr, g_scr_unused, ot_scr):
    rows = lax.broadcasted_iota(jnp.int32, (128, BQ), 0)
    qcols = pl.ds(q0, BQ)

    def head(h, carry):
        br = h // H
        slab = h // 4
        j = h % 4
        qrow = pl.multiple_of((slab % 4) * SLAB, 16)
        qs = qt_scr[br, pl.ds(qrow, 128), qcols].astype(f32)
        own = (rows >= j * DH) & (rows < (j + 1) * DH)
        vrow = pl.multiple_of(h * HP, HP)
        if fast:
            negm = -m_scr[pl.ds(h, 1), qcols]
            qw = jnp.where(own, qs, jnp.where(rows == AUG, negm, 0.0)).astype(bf16)
            acc = jnp.zeros((HP, BQ), f32)
            for c in range(0, S, CK):
                s = _mm(k_scr[slab, c:c + CK, :], qw)
                p = jnp.exp2(s).astype(bf16)
                acc = acc + _mm(vt_scr[pl.ds(vrow, HP), c:c + CK], p)
        else:
            qw = jnp.where(own, qs, 0.0).astype(bf16)

            def cmax(c, m8):
                s = _mm(k_scr[slab, pl.ds(pl.multiple_of(c * CKS, CKS), CKS), :], qw)
                return jnp.maximum(m8, jnp.max(s.reshape(CKS // 8, 8, BQ), axis=0))

            m8 = lax.fori_loop(0, S // CKS, cmax, jnp.full((8, BQ), -jnp.inf, f32))
            m = jnp.max(m8, axis=0, keepdims=True)

            def cacc(c, acc):
                cs = pl.ds(pl.multiple_of(c * CKS, CKS), CKS)
                s = _mm(k_scr[slab, cs, :], qw)
                p = jnp.exp2(s - m).astype(bf16)
                return acc + _mm(vt_scr[pl.ds(vrow, HP), cs], p)

            acc = lax.fori_loop(0, S // CKS, cacc, jnp.zeros((HP, BQ), f32))
        l = acc[DH:DH + 1, :]
        scale = g_scr[br, 0:1, qcols] / l
        ot_scr[pl.ds(vrow, HP), :] = (acc * scale).astype(bf16)
        lo, hi = carry
        return jnp.minimum(lo, l), jnp.maximum(hi, l)

    one = jnp.ones((1, BQ), f32)
    return lax.fori_loop(0, NH, head, (one, one))


def _kernel(x_ref, wa_ref, woa_ref, wb_ref, wob_ref, gw_ref, out_ref,
            qt_scr, k_scr, vt_scr, wot_scr, m_scr, g_scr, wt_scr, ot_scr):
    step = pl.program_id(0)

    @pl.when(step == 0)
    def _():
        _prologue(x_ref, (wa_ref, wb_ref), (woa_ref, wob_ref), gw_ref,
                  qt_scr, k_scr, vt_scr, wot_scr, m_scr, g_scr, wt_scr)

    q0 = pl.multiple_of(step * BQ, BQ)
    args = (q0, qt_scr, k_scr, vt_scr, m_scr, g_scr, None, ot_scr)
    lo, hi = _attend(True, *args)
    ok = jnp.where((lo >= L_MIN) & (hi <= L_MAX), 1.0, 0.0)
    safe = jnp.min(ok) > 0.5

    @pl.when(jnp.logical_not(safe))
    def _():
        _attend(False, *args)

    outt = _mm(wot_scr[...], ot_scr[...])
    out_ref[...] = outt.astype(out_ref.dtype)


@jax.jit
def pallas_gated_mix__mha_block__softmax_full_mha__prompt_kernel(
    A_x: jax.Array,
    A_wqkv: jax.Array,
    A_wo: jax.Array,
    B_x: jax.Array,
    B_wqkv: jax.Array,
    B_wo: jax.Array,
    gate_w: jax.Array,
):
    del B_x
    x = A_x.reshape(S, D).T
    gw = gate_w
    whole = lambda shape: pl.BlockSpec(shape, lambda i: (0,) * len(shape))
    out = pl.pallas_call(
        _kernel,
        grid=(S // BQ,),
        in_specs=[whole((D, S)), whole((D, 3 * D)), whole((D, D)), whole((D, 3 * D)), whole((D, D)),
                  whole((D,))],
        out_specs=pl.BlockSpec((D, BQ), lambda i: (0, i)),
        out_shape=jax.ShapeDtypeStruct((D, S), A_x.dtype),
        scratch_shapes=[
            pltpu.VMEM((2, QROWS, S), bf16),
            pltpu.VMEM((8, S, 128), bf16),
            pltpu.VMEM((NH * HP, S), bf16),
            pltpu.VMEM((D, NH * HP), bf16),
            pltpu.VMEM((NH, S), f32),
            pltpu.VMEM((2, 8, S), f32),
            pltpu.VMEM((2 * D + H * HP, D), bf16),
            pltpu.VMEM((NH * HP, BQ), bf16),
        ],
        compiler_params=pltpu.CompilerParams(
            dimension_semantics=("arbitrary",), vmem_limit_bytes=100 * 2 ** 20),
    )(x, A_wqkv, A_wo, B_wqkv, B_wo, gw)
    return out.T.reshape(A_x.shape)
```

```python
import jax
import jax.numpy as jnp
import numpy as np
from jax import lax
import jax.experimental.pallas as pl
import jax.experimental.pallas.tpu as pltpu

S = 2048
D = 448
H = 16
DH = 28
HP = 32
NH = 2 * H
SLAB = 4 * DH
AUG = SLAB
BQ = 2048
CK = 512
CKS = 256
TC = 512
TO = 256
QROWS = D + 16
HOOK_B = 1
HOOK_O = 2
WOFF = 16
WSPLIT = 512
LOG2E = float(np.log2(np.e))
QSCALE = float(DH ** -0.5) * LOG2E
L_MIN = float(2.0 ** -40)
L_MAX = float(2.0 ** 20)

bf16 = jnp.bfloat16
f32 = jnp.float32


def _mm(a, b):
    return jnp.dot(a, b, preferred_element_type=f32)


def _project_q(br, x_buf, wt, qt_scr, m_scr, g_scr, hook):
    lo = 0 if br == 0 else WOFF
    for t in range(0, S, TC):
        hook(t // TC)
        r = _mm(wt[lo:WOFF + D, :], x_buf[:, t:t + TC])
        if br == 0:
            g = 1.0 / (1.0 + jnp.exp(-r[0:8]))
            g_scr[0, :, t:t + TC] = g
            g_scr[1, :, t:t + TC] = 1.0 - g
            r = r[WOFF:]
        qt = r * QSCALE
        qt_scr[br, 0:D, t:t + TC] = qt.astype(bf16)
        q2 = qt * qt
        ns = [jnp.sum(q2[DH * h:DH * (h + 1)], axis=0, keepdims=True) for h in range(H)]
        m_scr[br * H:(br + 1) * H, t:t + TC] = jnp.concatenate(ns, axis=0)


def _project_kv(br, x_buf, wt, k_scr, vt_scr, m_scr, hook):
    row_k = lax.broadcasted_iota(jnp.int32, (128, TC), 0)
    tail_v = jnp.where(lax.broadcasted_iota(jnp.int32, (HP - DH, TC), 0) == 0, 1.0, 0.0)
    tail_k = jnp.zeros((16, TC), f32)
    kmax = [None] * H
    for t in range(0, S, TC):
        hook(t // TC)
        xt = x_buf[:, t:t + TC]
        kv = _mm(wt[WOFF + D:WOFF + 3 * D, :], xt)
        kt = kv[0:D]
        k2 = kt * kt
        for h in range(H):
            n2 = jnp.sum(k2[DH * h:DH * (h + 1)], axis=0, keepdims=True)
            kmax[h] = n2 if kmax[h] is None else jnp.maximum(kmax[h], n2)
        for s in range(4):
            slab = kt[SLAB * s:SLAB * s + 128] if s < 3 else jnp.concatenate([kt[SLAB * s:], tail_k], 0)
            slab = jnp.where(row_k == AUG, 1.0, slab)
            k_scr[br * 4 + s, t:t + TC, :] = slab.T.astype(bf16)
        parts = []
        for h in range(H):
            parts += [kv[D + DH * h:D + DH * (h + 1)], tail_v]
        vt_scr[br * H * HP:(br + 1) * H * HP, t:t + TC] = jnp.concatenate(parts, axis=0).astype(bf16)
    kcol = jnp.concatenate([jnp.max(k, axis=1, keepdims=True) for k in kmax], axis=0)
    rows = slice(br * H, (br + 1) * H)
    m_scr[rows, :] = jnp.sqrt(m_scr[rows, :] * kcol) * (1.0 + 2.0 ** -6)


def _attend(fast, q0, qt_scr, k_scr, vt_scr, m_scr, l_scr, ot_scr):
    rows = lax.broadcasted_iota(jnp.int32, (128, BQ), 0)
    qcols = pl.ds(q0, BQ)

    def head(h):
        br = h // H
        slab = h // 4
        j = h % 4
        qrow = pl.multiple_of((slab % 4) * SLAB, 16)
        qs = qt_scr[br, pl.ds(qrow, 128), qcols].astype(f32)
        own = (rows >= j * DH) & (rows < (j + 1) * DH)
        vrow = pl.multiple_of(h * HP, HP)
        if fast:
            qw = jnp.where(own, qs, jnp.where(rows == AUG, -m_scr[pl.ds(h, 1), qcols], 0.0)).astype(bf16)
            acc = None
            for c in range(0, S, CK):
                s = _mm(k_scr[slab, c:c + CK, :], qw)
                p = jnp.exp2(s).astype(bf16)
                o = _mm(vt_scr[pl.ds(vrow, HP), c:c + CK], p)
                acc = o if acc is None else acc + o
        else:
            qw = jnp.where(own, qs, 0.0).astype(bf16)

            def cmax(c, m8):
                s = _mm(k_scr[slab, pl.ds(pl.multiple_of(c * CKS, CKS), CKS), :], qw)
                return jnp.maximum(m8, jnp.max(s.reshape(CKS // 8, 8, BQ), axis=0))

            m8 = lax.fori_loop(0, S // CKS, cmax, jnp.full((8, BQ), -jnp.inf, f32))
            m = jnp.max(m8, axis=0, keepdims=True)

            def cacc(c, acc):
                cs = pl.ds(pl.multiple_of(c * CKS, CKS), CKS)
                s = _mm(k_scr[slab, cs, :], qw)
                p = jnp.exp2(s - m).astype(bf16)
                return acc + _mm(vt_scr[pl.ds(vrow, HP), cs], p)

            acc = lax.fori_loop(0, S // CKS, cacc, jnp.zeros((HP, BQ), f32))
        l_scr[pl.ds(h, 1), :] = acc[DH:DH + 1, :]
        return acc[0:DH]

    def pair(i, carry):
        oa = head(2 * i)
        ob = head(2 * i + 1)
        ot_scr[pl.ds(pl.multiple_of(i * 2 * DH, 8), 2 * DH), :] = jnp.concatenate([oa, ob], axis=0)
        return carry

    lax.fori_loop(0, NH // 2, pair, 0)


def _kernel(x_hbm, wa_hbm, woa_hbm, wb_hbm, wob_hbm, gw_hbm, out_hbm,
            x_buf, wa_buf, wb_buf, woa_buf, wob_buf, gw_buf, out_buf,
            qt_scr, k_scr, vt_scr, wot_scr, m_scr, g_scr, wta, wtb, ot_scr, l_scr,
            sem_in, sem_x, sem_out):
    nx = S // TC
    W0 = pl.ds(0, WSPLIT)
    W1 = pl.ds(WSPLIT, 3 * D - WSPLIT)
    cp_wa0 = pltpu.make_async_copy(wa_hbm.at[:, W0], wa_buf.at[:, W0], sem_in.at[0])
    cp_wa1 = pltpu.make_async_copy(wa_hbm.at[:, W1], wa_buf.at[:, W1], sem_in.at[5])
    cp_wb = pltpu.make_async_copy(wb_hbm, wb_buf, sem_in.at[1])
    cp_woa = pltpu.make_async_copy(woa_hbm, woa_buf, sem_in.at[2])
    cp_wob = pltpu.make_async_copy(wob_hbm, wob_buf, sem_in.at[3])
    cp_gw = pltpu.make_async_copy(gw_hbm, gw_buf, sem_in.at[4])
    cp_x = [pltpu.make_async_copy(x_hbm.at[:, pl.ds(i * TC, TC)], x_buf.at[:, pl.ds(i * TC, TC)], sem_x.at[i])
            for i in range(nx)]
    cp_gw.start()
    cp_wa0.start()
    cp_x[0].start()
    cp_gw.wait()
    cp_wa0.wait()
    cp_wa1.start()

    def hook_qa(i):
        cp_x[i].wait()
        if i + 1 < nx:
            cp_x[i + 1].start()
        else:
            cp_wb.start()

    def hook_kva(i):
        if i == 0:
            cp_woa.start()
            cp_wob.start()
        if i == HOOK_B:
            cp_wb.wait()
            wtb[WOFF:, :] = wb_buf[...].T
        if i == HOOK_O:
            cp_woa.wait()
            cp_wob.wait()
            wot_scr[...] = jnp.concatenate([woa_buf[...], wob_buf[...]], axis=0).T

    qt_scr[:, D:QROWS, :] = jnp.zeros((2, QROWS - D, S), bf16)
    wta[0:WOFF, :] = jnp.broadcast_to(gw_buf[...].reshape(1, D), (WOFF, D))
    wta[WOFF:WOFF + WSPLIT, :] = wa_buf[:, 0:WSPLIT].T
    _project_q(0, x_buf, wta, qt_scr, m_scr, g_scr, hook_qa)
    cp_wa1.wait()
    wta[WOFF + WSPLIT:, :] = wa_buf[:, WSPLIT:].T
    _project_kv(0, x_buf, wta, k_scr, vt_scr, m_scr, hook_kva)
    _project_q(1, x_buf, wtb, qt_scr, m_scr, g_scr, lambda i: None)
    _project_kv(1, x_buf, wtb, k_scr, vt_scr, m_scr, lambda i: None)

    n_out = 0
    for q0 in range(0, S, BQ):
        args = (q0, qt_scr, k_scr, vt_scr, m_scr, l_scr, ot_scr)
        _attend(True, *args)
        l = l_scr[...]
        safe = jnp.min(jnp.where((l >= L_MIN) & (l <= L_MAX), 1.0, 0.0)) > 0.5

        @pl.when(jnp.logical_not(safe))
        def _():
            _attend(False, *args)

        for t in range(0, BQ, TO):
            tc = slice(t, t + TO)
            qc = slice(q0 + t, q0 + t + TO)
            gate = jnp.concatenate([jnp.broadcast_to(g_scr[0, 0:1, qc], (H, TO)),
                                    jnp.broadcast_to(g_scr[1, 0:1, qc], (H, TO))], axis=0)
            sc = gate / l_scr[:, tc]
            sc = jnp.concatenate([jnp.broadcast_to(sc[h:h + 1], (DH, TO)) for h in range(NH)], axis=0)
            o = (ot_scr[:, tc] * sc).astype(bf16)
            out_buf[:, qc] = _mm(wot_scr[...], o).astype(bf16)
            pltpu.make_async_copy(out_buf.at[:, qc], out_hbm.at[:, qc], sem_out.at[n_out]).start()
            n_out += 1
    for i in range(n_out):
        pltpu.make_async_copy(out_buf.at[:, pl.ds(i * TO, TO)], out_hbm.at[:, pl.ds(i * TO, TO)],
                              sem_out.at[i]).wait()


@jax.jit
def pallas_gated_mix__mha_block__softmax_full_mha__prompt_kernel(
    A_x: jax.Array,
    A_wqkv: jax.Array,
    A_wo: jax.Array,
    B_x: jax.Array,
    B_wqkv: jax.Array,
    B_wo: jax.Array,
    gate_w: jax.Array,
):
    del B_x
    x = A_x.reshape(S, D).T
    hbm = pl.BlockSpec(memory_space=pl.ANY)
    out = pl.pallas_call(
        _kernel,
        in_specs=[hbm] * 6,
        out_specs=hbm,
        out_shape=jax.ShapeDtypeStruct((D, S), A_x.dtype),
        scratch_shapes=[
            pltpu.VMEM((D, S), bf16),
            pltpu.VMEM((D, 3 * D), bf16),
            pltpu.VMEM((D, 3 * D), bf16),
            pltpu.VMEM((D, D), bf16),
            pltpu.VMEM((D, D), bf16),
            pltpu.VMEM((D,), bf16),
            pltpu.VMEM((D, S), bf16),
            pltpu.VMEM((2, QROWS, S), bf16),
            pltpu.VMEM((8, S, 128), bf16),
            pltpu.VMEM((NH * HP, S), bf16),
            pltpu.VMEM((D, 2 * D), bf16),
            pltpu.VMEM((NH, S), f32),
            pltpu.VMEM((2, 8, S), f32),
            pltpu.VMEM((WOFF + 3 * D, D), bf16),
            pltpu.VMEM((WOFF + 3 * D, D), bf16),
            pltpu.VMEM((2 * D, BQ), f32),
            pltpu.VMEM((NH, BQ), f32),
            pltpu.SemaphoreType.DMA((6,)),
            pltpu.SemaphoreType.DMA((S // TC,)),
            pltpu.SemaphoreType.DMA((S // TO,)),
        ],
        compiler_params=pltpu.CompilerParams(vmem_limit_bytes=100 * 2 ** 20),
    )(x, A_wqkv, A_wo, B_wqkv, B_wo, gate_w)
    return out.T.reshape(A_x.shape)
```

```python
import jax
import jax.numpy as jnp
import numpy as np
from jax import lax
import jax.experimental.pallas as pl
import jax.experimental.pallas.tpu as pltpu

S = 2048
D = 448
H = 16
DH = 28
HP = 32
NH = 2 * H
SLAB = 4 * DH
AUG = SLAB
CK = 512
CKS = 256
TC = 512
TO = 256
QROWS = D + 16
WOFF = 16
WSPLIT = 512
QSCALE = float(DH ** -0.5 * np.log2(np.e))
M_SLACK = 1.0 + 2.0 ** -6
L_MIN = float(2.0 ** -40)
L_MAX = float(2.0 ** 20)

bf16 = jnp.bfloat16
f32 = jnp.float32


def _mm(a, b):
    return jnp.dot(a, b, preferred_element_type=f32)


def _head_sums(v):
    return jnp.concatenate(
        [jnp.sum(v[DH * h:DH * (h + 1)], axis=0, keepdims=True) for h in range(H)], axis=0)


def _project_q(br, x_buf, wt, qt_scr, m_scr, g_scr, hook):
    lo = 0 if br == 0 else WOFF
    for t in range(0, S, TC):
        hook(t // TC)
        r = _mm(wt[lo:WOFF + D, :], x_buf[:, t:t + TC])
        if br == 0:
            g = 1.0 / (1.0 + jnp.exp(-r[0:8]))
            g_scr[0, :, t:t + TC] = g
            g_scr[1, :, t:t + TC] = 1.0 - g
            r = r[WOFF:]
        qt = r * QSCALE
        qt_scr[br, 0:D, t:t + TC] = qt.astype(bf16)
        m_scr[br * H:(br + 1) * H, t:t + TC] = _head_sums(qt * qt)


def _project_kv(br, x_buf, wt, k_scr, vt_scr, m_scr, hook):
    row_k = lax.broadcasted_iota(jnp.int32, (128, TC), 0)
    tail_v = jnp.where(lax.broadcasted_iota(jnp.int32, (HP - DH, TC), 0) == 0, 1.0, 0.0)
    tail_k = jnp.zeros((16, TC), f32)
    kmax = None
    for t in range(0, S, TC):
        hook(t // TC)
        kv = _mm(wt[WOFF + D:WOFF + 3 * D, :], x_buf[:, t:t + TC])
        kt = kv[0:D]
        n2 = _head_sums(kt * kt)
        kmax = n2 if kmax is None else jnp.maximum(kmax, n2)
        for s in range(4):
            slab = kt[SLAB * s:SLAB * s + 128] if s < 3 else jnp.concatenate([kt[SLAB * s:], tail_k], 0)
            slab = jnp.where(row_k == AUG, 1.0, slab)
            k_scr[br * 4 + s, t:t + TC, :] = slab.T.astype(bf16)
        parts = []
        for h in range(H):
            parts += [kv[D + DH * h:D + DH * (h + 1)], tail_v]
        vt_scr[br * H * HP:(br + 1) * H * HP, t:t + TC] = jnp.concatenate(parts, axis=0).astype(bf16)
    kcol = jnp.max(kmax, axis=1, keepdims=True)
    rows = slice(br * H, (br + 1) * H)
    m_scr[rows, :] = jnp.sqrt(m_scr[rows, :] * kcol) * -M_SLACK


def _attend(fast, qt_scr, k_scr, vt_scr, m_scr, l_scr, ot_scr):
    rows = lax.broadcasted_iota(jnp.int32, (128, S), 0)

    def head(h):
        slab = h >> 2
        qrow = pl.multiple_of((slab & 3) * SLAB, 16)
        qs = qt_scr[h >> 4, pl.ds(qrow, 128), :].astype(f32)
        first = (h & 3) * DH
        own = (rows >= first) & (rows < first + DH)
        vrow = pl.multiple_of(h * HP, HP)
        if fast:
            qw = jnp.where(own, qs, jnp.where(rows == AUG, m_scr[pl.ds(h, 1), :], 0.0)).astype(bf16)
            acc = None
            for c in range(0, S, CK):
                s = _mm(k_scr[slab, c:c + CK, :], qw)
                p = jnp.exp2(s).astype(bf16)
                o = _mm(vt_scr[pl.ds(vrow, HP), c:c + CK], p)
                acc = o if acc is None else acc + o
        else:
            qw = jnp.where(own, qs, 0.0).astype(bf16)

            def cmax(c, m8):
                s = _mm(k_scr[slab, pl.ds(pl.multiple_of(c * CKS, CKS), CKS), :], qw)
                return jnp.maximum(m8, jnp.max(s.reshape(CKS // 8, 8, S), axis=0))

            m8 = lax.fori_loop(0, S // CKS, cmax, jnp.full((8, S), -jnp.inf, f32))
            m = jnp.max(m8, axis=0, keepdims=True)

            def cacc(c, acc):
                cs = pl.ds(pl.multiple_of(c * CKS, CKS), CKS)
                s = _mm(k_scr[slab, cs, :], qw)
                p = jnp.exp2(s - m).astype(bf16)
                return acc + _mm(vt_scr[pl.ds(vrow, HP), cs], p)

            acc = lax.fori_loop(0, S // CKS, cacc, jnp.zeros((HP, S), f32))
        l_scr[pl.ds(h, 1), :] = acc[DH:DH + 1, :]
        return acc[0:DH]

    def pair(i, carry):
        oa = head(2 * i)
        ob = head(2 * i + 1)
        ot_scr[pl.ds(pl.multiple_of(i * 2 * DH, 8), 2 * DH), :] = jnp.concatenate([oa, ob], axis=0)
        return carry

    lax.fori_loop(0, NH // 2, pair, 0)


def _kernel(x_hbm, wa_hbm, woa_hbm, wb_hbm, wob_hbm, gw_hbm, out_hbm,
            x_buf, wa_buf, wb_buf, woa_buf, wob_buf, gw_buf, out_buf,
            qt_scr, k_scr, vt_scr, wot_scr, m_scr, g_scr, wta, wtb, ot_scr, l_scr,
            sem_in, sem_x, sem_out):
    nx = S // TC
    w0 = pl.ds(0, WSPLIT)
    w1 = pl.ds(WSPLIT, 3 * D - WSPLIT)
    cp_wa0 = pltpu.make_async_copy(wa_hbm.at[:, w0], wa_buf.at[:, w0], sem_in.at[0])
    cp_wa1 = pltpu.make_async_copy(wa_hbm.at[:, w1], wa_buf.at[:, w1], sem_in.at[1])
    cp_wb = pltpu.make_async_copy(wb_hbm, wb_buf, sem_in.at[2])
    cp_woa = pltpu.make_async_copy(woa_hbm, woa_buf, sem_in.at[3])
    cp_wob = pltpu.make_async_copy(wob_hbm, wob_buf, sem_in.at[4])
    cp_gw = pltpu.make_async_copy(gw_hbm, gw_buf, sem_in.at[5])
    cp_x = [pltpu.make_async_copy(x_hbm.at[:, pl.ds(i * TC, TC)], x_buf.at[:, pl.ds(i * TC, TC)], sem_x.at[i])
            for i in range(nx)]

    cp_gw.start()
    cp_wa0.start()
    cp_x[0].start()
    cp_gw.wait()
    cp_wa0.wait()
    cp_wa1.start()

    def hook_qa(i):
        cp_x[i].wait()
        if i + 1 < nx:
            cp_x[i + 1].start()
        else:
            cp_wb.start()

    def hook_kva(i):
        if i == 0:
            cp_woa.start()
            cp_wob.start()
        if i == 1:
            cp_wb.wait()
            wtb[WOFF:, :] = wb_buf[...].T
        if i == 2:
            cp_woa.wait()
            cp_wob.wait()
            wot_scr[...] = jnp.concatenate([woa_buf[...], wob_buf[...]], axis=0).T

    def no_hook(i):
        pass

    qt_scr[:, D:QROWS, :] = jnp.zeros((2, QROWS - D, S), bf16)
    wta[0:WOFF, :] = jnp.broadcast_to(gw_buf[...].reshape(1, D), (WOFF, D))
    wta[WOFF:WOFF + WSPLIT, :] = wa_buf[:, 0:WSPLIT].T
    _project_q(0, x_buf, wta, qt_scr, m_scr, g_scr, hook_qa)
    cp_wa1.wait()
    wta[WOFF + WSPLIT:, :] = wa_buf[:, WSPLIT:].T
    _project_kv(0, x_buf, wta, k_scr, vt_scr, m_scr, hook_kva)
    _project_q(1, x_buf, wtb, qt_scr, m_scr, g_scr, no_hook)
    _project_kv(1, x_buf, wtb, k_scr, vt_scr, m_scr, no_hook)

    args = (qt_scr, k_scr, vt_scr, m_scr, l_scr, ot_scr)
    _attend(True, *args)
    l = l_scr[...]
    safe = jnp.min(jnp.where((l >= L_MIN) & (l <= L_MAX), 1.0, 0.0)) > 0.5

    @pl.when(jnp.logical_not(safe))
    def _():
        _attend(False, *args)

    cp_out = []
    for t in range(0, S, TO):
        tc = slice(t, t + TO)
        gate = jnp.concatenate([jnp.broadcast_to(g_scr[0, 0:1, tc], (H, TO)),
                                jnp.broadcast_to(g_scr[1, 0:1, tc], (H, TO))], axis=0)
        sc = gate / l_scr[:, tc]
        sc = jnp.concatenate([jnp.broadcast_to(sc[h:h + 1], (DH, TO)) for h in range(NH)], axis=0)
        o = (ot_scr[:, tc] * sc).astype(bf16)
        out_buf[:, tc] = _mm(wot_scr[...], o).astype(bf16)
        cp_out.append(pltpu.make_async_copy(
            out_buf.at[:, pl.ds(t, TO)], out_hbm.at[:, pl.ds(t, TO)], sem_out.at[t // TO]))
        cp_out[-1].start()
    for c in cp_out:
        c.wait()


@jax.jit
def pallas_gated_mix__mha_block__softmax_full_mha__prompt_kernel(
    A_x: jax.Array,
    A_wqkv: jax.Array,
    A_wo: jax.Array,
    B_x: jax.Array,
    B_wqkv: jax.Array,
    B_wo: jax.Array,
    gate_w: jax.Array,
):
    del B_x
    xt = A_x.reshape(S, D).T
    hbm = pl.BlockSpec(memory_space=pl.ANY)
    out = pl.pallas_call(
        _kernel,
        in_specs=[hbm] * 6,
        out_specs=hbm,
        out_shape=jax.ShapeDtypeStruct((D, S), A_x.dtype),
        scratch_shapes=[
            pltpu.VMEM((D, S), bf16),
            pltpu.VMEM((D, 3 * D), bf16),
            pltpu.VMEM((D, 3 * D), bf16),
            pltpu.VMEM((D, D), bf16),
            pltpu.VMEM((D, D), bf16),
            pltpu.VMEM((D,), bf16),
            pltpu.VMEM((D, S), bf16),
            pltpu.VMEM((2, QROWS, S), bf16),
            pltpu.VMEM((8, S, 128), bf16),
            pltpu.VMEM((NH * HP, S), bf16),
            pltpu.VMEM((D, 2 * D), bf16),
            pltpu.VMEM((NH, S), f32),
            pltpu.VMEM((2, 8, S), f32),
            pltpu.VMEM((WOFF + 3 * D, D), bf16),
            pltpu.VMEM((WOFF + 3 * D, D), bf16),
            pltpu.VMEM((2 * D, S), f32),
            pltpu.VMEM((NH, S), f32),
            pltpu.SemaphoreType.DMA((6,)),
            pltpu.SemaphoreType.DMA((S // TC,)),
            pltpu.SemaphoreType.DMA((S // TO,)),
        ],
        compiler_params=pltpu.CompilerParams(vmem_limit_bytes=100 * 2 ** 20),
    )(xt, A_wqkv, A_wo, B_wqkv, B_wo, gate_w)
    return out.T.reshape(A_x.shape)
```

```python
import jax
import jax.numpy as jnp
import numpy as np
from jax import lax
import jax.experimental.pallas as pl
import jax.experimental.pallas.tpu as pltpu

S = 2048
D = 448
H = 16
DH = 28
HP = 32
NH = 2 * H
SLAB = 4 * DH
AUG = SLAB
CK = 512
CKS = 256
TC = 512
TO = 256
QROWS = D + 16
WOFF = 16
WCUT = (0, 128, 512, 3 * D)
QSCALE = float(DH ** -0.5 * np.log2(np.e))
M_SLACK = 1.0 + 2.0 ** -6
L_MIN = float(2.0 ** -40)
L_MAX = float(2.0 ** 20)

bf16 = jnp.bfloat16
f32 = jnp.float32


def _mm(a, b):
    return jnp.dot(a, b, preferred_element_type=f32)


def _head_sums(v):
    return jnp.concatenate(
        [jnp.sum(v[DH * h:DH * (h + 1)], axis=0, keepdims=True) for h in range(H)], axis=0)


def _project_q(br, x_buf, wt, qt_scr, m_scr, g_scr, hook):
    lo = 0 if br == 0 else WOFF
    for t in range(0, S, TC):
        hook(t // TC)
        if br == 0 and t == 0:
            r0 = _mm(wt[0:WOFF + WCUT[1], :], x_buf[:, 0:TC])
            hook(-1)
            r = jnp.concatenate([r0, _mm(wt[WOFF + WCUT[1]:WOFF + D, :], x_buf[:, 0:TC])], axis=0)
        else:
            r = _mm(wt[lo:WOFF + D, :], x_buf[:, t:t + TC])
        if br == 0:
            g = 1.0 / (1.0 + jnp.exp(-r[0:8]))
            g_scr[0, :, t:t + TC] = g
            g_scr[1, :, t:t + TC] = 1.0 - g
            r = r[WOFF:]
        qt = r * QSCALE
        qt_scr[br, 0:D, t:t + TC] = qt.astype(bf16)
        m_scr[br * H:(br + 1) * H, t:t + TC] = _head_sums(qt * qt)


def _project_kv(br, x_buf, wt, k_scr, vt_scr, m_scr, hook):
    row_k = lax.broadcasted_iota(jnp.int32, (128, TC), 0)
    tail_v = jnp.where(lax.broadcasted_iota(jnp.int32, (HP - DH, TC), 0) == 0, 1.0, 0.0)
    tail_k = jnp.zeros((16, TC), f32)
    kmax = None
    for t in range(0, S, TC):
        hook(t // TC)
        kv = _mm(wt[WOFF + D:WOFF + 3 * D, :], x_buf[:, t:t + TC])
        kt = kv[0:D]
        n2 = _head_sums(kt * kt)
        kmax = n2 if kmax is None else jnp.maximum(kmax, n2)
        for s in range(4):
            slab = kt[SLAB * s:SLAB * s + 128] if s < 3 else jnp.concatenate([kt[SLAB * s:], tail_k], 0)
            slab = jnp.where(row_k == AUG, 1.0, slab)
            k_scr[br * 4 + s, t:t + TC, :] = slab.T.astype(bf16)
        parts = []
        for h in range(H):
            parts += [kv[D + DH * h:D + DH * (h + 1)], tail_v]
        vt_scr[br * H * HP:(br + 1) * H * HP, t:t + TC] = jnp.concatenate(parts, axis=0).astype(bf16)
    kcol = jnp.max(kmax, axis=1, keepdims=True)
    rows = slice(br * H, (br + 1) * H)
    m_scr[rows, :] = jnp.sqrt(m_scr[rows, :] * kcol) * -M_SLACK


def _q_operand(h, qs, rows, aug):
    first = (h & 3) * DH
    own = (rows >= first) & (rows < first + DH)
    return jnp.where(own, qs, jnp.where(rows == AUG, aug, 0.0)).astype(bf16)


def _attend(fast, qt_scr, k_scr, vt_scr, m_scr, l_scr, ot_scr):
    rows = lax.broadcasted_iota(jnp.int32, (128, S), 0)

    def bounded(heads, slab, qs):
        qw = [_q_operand(h, qs, rows, m_scr[pl.ds(h, 1), :]) for h in heads]
        acc = [None, None]
        for c in range(0, S, CK):
            for e, h in enumerate(heads):
                p = jnp.exp2(_mm(k_scr[slab, c:c + CK, :], qw[e])).astype(bf16)
                o = _mm(vt_scr[pl.ds(pl.multiple_of(h * HP, HP), HP), c:c + CK], p)
                acc[e] = o if acc[e] is None else acc[e] + o
        return acc

    def exact(h, slab, qs):
        qw = _q_operand(h, qs, rows, 0.0)

        def scores(c):
            return _mm(k_scr[slab, pl.ds(pl.multiple_of(c * CKS, CKS), CKS), :], qw)

        def cmax(c, m8):
            return jnp.maximum(m8, jnp.max(scores(c).reshape(CKS // 8, 8, S), axis=0))

        m8 = lax.fori_loop(0, S // CKS, cmax, jnp.full((8, S), -jnp.inf, f32))
        m = jnp.max(m8, axis=0, keepdims=True)

        def cacc(c, acc):
            p = jnp.exp2(scores(c) - m).astype(bf16)
            return acc + _mm(vt_scr[pl.ds(pl.multiple_of(h * HP, HP), HP),
                                    pl.ds(pl.multiple_of(c * CKS, CKS), CKS)], p)

        return lax.fori_loop(0, S // CKS, cacc, jnp.zeros((HP, S), f32))

    def pair(i, carry):
        heads = (2 * i, 2 * i + 1)
        slab = i >> 1
        qs = qt_scr[i >> 3, pl.ds(pl.multiple_of((slab & 3) * SLAB, 16), 128), :].astype(f32)
        acc = bounded(heads, slab, qs) if fast else [exact(h, slab, qs) for h in heads]
        for h, a in zip(heads, acc):
            l_scr[pl.ds(h, 1), :] = a[DH:DH + 1, :]
        ot_scr[pl.ds(pl.multiple_of(i * 2 * DH, 8), 2 * DH), :] = jnp.concatenate(
            [acc[0][0:DH], acc[1][0:DH]], axis=0)
        return carry

    lax.fori_loop(0, NH // 2, pair, 0)


def _kernel(x_hbm, wa_hbm, woa_hbm, wb_hbm, wob_hbm, gw_hbm, out_hbm,
            x_buf, wa_buf, wb_buf, woa_buf, wob_buf, gw_buf, out_buf,
            qt_scr, k_scr, vt_scr, wot_scr, m_scr, g_scr, wta, wtb, ot_scr, l_scr,
            sem_in, sem_w, sem_x, sem_out):
    nx = S // TC
    cp_wa = [pltpu.make_async_copy(wa_hbm.at[:, pl.ds(a, b - a)], wa_buf.at[:, pl.ds(a, b - a)], sem_w.at[k])
             for k, (a, b) in enumerate(zip(WCUT[:-1], WCUT[1:]))]
    cp_wb = pltpu.make_async_copy(wb_hbm, wb_buf, sem_in.at[0])
    cp_woa = pltpu.make_async_copy(woa_hbm, woa_buf, sem_in.at[1])
    cp_wob = pltpu.make_async_copy(wob_hbm, wob_buf, sem_in.at[2])
    cp_gw = pltpu.make_async_copy(gw_hbm, gw_buf, sem_in.at[3])
    cp_x = [pltpu.make_async_copy(x_hbm.at[:, pl.ds(i * TC, TC)], x_buf.at[:, pl.ds(i * TC, TC)], sem_x.at[i])
            for i in range(nx)]

    cp_gw.start()
    cp_wa[0].start()
    cp_x[0].start()
    cp_wa[1].start()
    cp_gw.wait()

    def land_wa(k):
        cp_wa[k].wait()
        if k == 1:
            cp_wa[2].start()
        wta[WOFF + WCUT[k]:WOFF + WCUT[k + 1], :] = wa_buf[:, WCUT[k]:WCUT[k + 1]].T

    def hook_qa(i):
        if i < 0:
            land_wa(1)
            return
        if i == 0:
            land_wa(0)
        cp_x[i].wait()
        if i + 1 < nx:
            cp_x[i + 1].start()
        else:
            cp_wb.start()

    def hook_kva(i):
        if i == 0:
            cp_woa.start()
            cp_wob.start()
        if i == 1:
            cp_wb.wait()
            wtb[WOFF:, :] = wb_buf[...].T
        if i == 2:
            cp_woa.wait()
            cp_wob.wait()
            wot_scr[...] = jnp.concatenate([woa_buf[...], wob_buf[...]], axis=0).T

    def no_hook(i):
        pass

    qt_scr[:, D:QROWS, :] = jnp.zeros((2, QROWS - D, S), bf16)
    wta[0:WOFF, :] = jnp.broadcast_to(gw_buf[...].reshape(1, D), (WOFF, D))
    _project_q(0, x_buf, wta, qt_scr, m_scr, g_scr, hook_qa)
    land_wa(2)
    _project_kv(0, x_buf, wta, k_scr, vt_scr, m_scr, hook_kva)
    _project_q(1, x_buf, wtb, qt_scr, m_scr, g_scr, no_hook)
    _project_kv(1, x_buf, wtb, k_scr, vt_scr, m_scr, no_hook)

    args = (qt_scr, k_scr, vt_scr, m_scr, l_scr, ot_scr)
    _attend(True, *args)
    l = l_scr[...]
    safe = jnp.min(jnp.where((l >= L_MIN) & (l <= L_MAX), 1.0, 0.0)) > 0.5

    @pl.when(jnp.logical_not(safe))
    def _():
        _attend(False, *args)

    cp_out = []
    for t in range(0, S, TO):
        tc = slice(t, t + TO)
        gate = jnp.concatenate([jnp.broadcast_to(g_scr[0, 0:1, tc], (H, TO)),
                                jnp.broadcast_to(g_scr[1, 0:1, tc], (H, TO))], axis=0)
        sc = gate / l_scr[:, tc]
        sc = jnp.concatenate([jnp.broadcast_to(sc[h:h + 1], (DH, TO)) for h in range(NH)], axis=0)
        o = (ot_scr[:, tc] * sc).astype(bf16)
        out_buf[:, tc] = _mm(wot_scr[...], o).astype(bf16)
        cp_out.append(pltpu.make_async_copy(
            out_buf.at[:, pl.ds(t, TO)], out_hbm.at[:, pl.ds(t, TO)], sem_out.at[t // TO]))
        cp_out[-1].start()
    for c in cp_out:
        c.wait()


@jax.jit
def pallas_gated_mix__mha_block__softmax_full_mha__prompt_kernel(
    A_x: jax.Array,
    A_wqkv: jax.Array,
    A_wo: jax.Array,
    B_x: jax.Array,
    B_wqkv: jax.Array,
    B_wo: jax.Array,
    gate_w: jax.Array,
):
    del B_x
    xt = A_x.reshape(S, D).T
    hbm = pl.BlockSpec(memory_space=pl.ANY)
    out = pl.pallas_call(
        _kernel,
        in_specs=[hbm] * 6,
        out_specs=hbm,
        out_shape=jax.ShapeDtypeStruct((D, S), A_x.dtype),
        scratch_shapes=[
            pltpu.VMEM((D, S), bf16),
            pltpu.VMEM((D, 3 * D), bf16),
            pltpu.VMEM((D, 3 * D), bf16),
            pltpu.VMEM((D, D), bf16),
            pltpu.VMEM((D, D), bf16),
            pltpu.VMEM((D,), bf16),
            pltpu.VMEM((D, S), bf16),
            pltpu.VMEM((2, QROWS, S), bf16),
            pltpu.VMEM((8, S, 128), bf16),
            pltpu.VMEM((NH * HP, S), bf16),
            pltpu.VMEM((D, 2 * D), bf16),
            pltpu.VMEM((NH, S), f32),
            pltpu.VMEM((2, 8, S), f32),
            pltpu.VMEM((WOFF + 3 * D, D), bf16),
            pltpu.VMEM((WOFF + 3 * D, D), bf16),
            pltpu.VMEM((2 * D, S), f32),
            pltpu.VMEM((NH, S), f32),
            pltpu.SemaphoreType.DMA((4,)),
            pltpu.SemaphoreType.DMA((3,)),
            pltpu.SemaphoreType.DMA((S // TC,)),
            pltpu.SemaphoreType.DMA((S // TO,)),
        ],
        compiler_params=pltpu.CompilerParams(vmem_limit_bytes=100 * 2 ** 20),
    )(xt, A_wqkv, A_wo, B_wqkv, B_wo, gate_w)
    return out.T.reshape(A_x.shape)
```
